```python
import os as _os
_os.environ.setdefault("JAX_PLATFORMS", "cpu")
import jax
import jax.numpy as jnp

def _softmax(x, axis=-1):
    return jax.nn.softmax(x, axis=axis)
def _gelu(x):
    return jax.nn.gelu(x, approximate=True)
def _silu(x):
    return jax.nn.silu(x)
def _sigmoid(x):
    return jax.nn.sigmoid(x)
def _layernorm(x, axis=-1, eps=1e-5):
    m = jnp.mean(x, axis=axis, keepdims=True)
    v = jnp.var(x, axis=axis, keepdims=True)
    return (x - m) / jnp.sqrt(v + eps)
def _scatter_add(tgt, idx, src, axis=0):
    return tgt.at[idx].add(src)
def _segment_sum(src, seg, n):
    return jax.ops.segment_sum(src, seg, n)
class _Rng:
    def __init__(self, key):
        self._k = key
    def _next(self):
        self._k, sub = jax.random.split(self._k)
        return sub
    def normal(self, shape):
        return jax.random.normal(self._next(), shape, dtype=jnp.bfloat16)
    def randint(self, lo, hi, shape):
        return jax.random.randint(self._next(), shape, lo, hi, dtype=jnp.int32)
    def uniform(self, shape, lo=0.0, hi=1.0):
        return jax.random.uniform(self._next(), shape, jnp.bfloat16, lo, hi)
    def permutation(self, n):
        return jax.random.permutation(self._next(), n)


kernel_name = 'standalone__linear_kernel_rfa__decode'

def setup_inputs():
    _rng = _Rng(jax.random.key(int.from_bytes(__import__("os").urandom(4), "little")))
    _w = (lambda a: (lambda t: t.astype(jnp.bfloat16) if jnp.issubdtype(t.dtype, jnp.floating) else t)(jnp.asarray(a)))
    B, H, Sq, Sk, D, M = 2, 16, 1, 16384, 256, 16
    return {
        "q": _w((lambda *s: _rng.normal(s) * 0.4)(B, H, Sq, D)),
        "k": _w((lambda *s: _rng.normal(s) * 1.6)(B, H, Sk, D)),
        "v": _w((lambda *s: _rng.normal(s) * 1.6)(B, H, Sk, D)),
        "omega": _w((lambda *s: _rng.normal(s) * 1.6)(M, D)),
    }

def reference(q, k, v, omega):
    d = q.shape[-1]
    m = omega.shape[0]
    scale = float(d) ** -0.25
    qs = q * scale
    ks = k * scale
    q_proj = jnp.einsum("bhsd,md->bhsm", qs, omega)
    k_proj = jnp.einsum("bhsd,md->bhsm", ks, omega)
    q_sq = 0.5 * jnp.einsum("bhsd,bhsd->bhs", qs, qs)[..., None]
    k_sq = 0.5 * jnp.einsum("bhsd,bhsd->bhs", ks, ks)[..., None]
    inv_sqrt_m = float(m) ** -0.5
    phi_q = jnp.exp(q_proj - q_sq) * inv_sqrt_m + 1e-6
    phi_k = jnp.exp(k_proj - k_sq) * inv_sqrt_m + 1e-6
    kv = jnp.einsum("bhsm,bhsd->bhmd", phi_k, v)
    z  = jnp.einsum("bhsm->bhm", phi_k)
    num = jnp.einsum("bhqm,bhmd->bhqd", phi_q, kv)
    den = jnp.einsum("bhqm,bhm->bhq", phi_q, z)[..., None] + 1e-6
    return num / den
```

```python
import jax
import jax.numpy as jnp
from jax import lax
import jax.experimental.pallas as pl
import jax.experimental.pallas.tpu as pltpu

_F32 = jnp.float32
_BF16 = jnp.bfloat16
_NT = (((1,), (1,)), ((), ()))


def _rb(x):
    return x.astype(_BF16).astype(_F32)


@jax.jit
def pallas_standalone__linear_kernel_rfa__decode_kernel(
    q: jax.Array,
    k: jax.Array,
    v: jax.Array,
    omega: jax.Array,
):
    B, H, Sq, D = q.shape
    S = k.shape[2]
    M = omega.shape[0]
    assert Sq == 1 and D == 256
    TS = 2048
    assert S % TS == 0
    scale = float(D) ** -0.25
    inv_sqrt_m = float(M) ** -0.5

    def kernel(q_ref, k_ref, v_ref, om_ref, o_ref, kv_acc, z_acc):
        j = pl.program_id(1)

        @pl.when(j == 0)
        def _():
            kv_acc[...] = jnp.zeros_like(kv_acc)
            z_acc[...] = jnp.zeros_like(z_acc)

        om = om_ref[...]
        kk = k_ref[...]
        kp = lax.dot_general(om, kk, _NT, preferred_element_type=_F32)
        kf = kk.astype(_F32)
        sq = kf * kf
        sh = sq[:, :128] + sq[:, 128:]
        ksq = jnp.sum(sh.T, axis=0, keepdims=True)
        kp = _rb(kp * scale)
        ksq = _rb(_rb(ksq * (scale * scale)) * 0.5)
        e = _rb(jnp.exp(_rb(kp - ksq)))
        phi = (_rb(e * inv_sqrt_m) + 1e-6).astype(_BF16)
        kv_acc[...] += jnp.dot(phi, v_ref[...], preferred_element_type=_F32)
        pf = phi.astype(_F32)
        zp = pf[:, 0:128]
        for t in range(1, TS // 128):
            zp = zp + pf[:, t * 128:(t + 1) * 128]
        z_acc[...] += zp

        @pl.when(j == pl.num_programs(1) - 1)
        def _():
            qs = q_ref[...].astype(_F32) * scale
            omf = om.astype(_F32)
            qp = _rb(jnp.sum(omf * qs, axis=1, keepdims=True))
            qsq = _rb(_rb(jnp.sum(qs * qs, axis=1, keepdims=True)) * 0.5)
            eq = _rb(jnp.exp(_rb(qp - qsq)))
            phq = _rb(_rb(eq * inv_sqrt_m) + 1e-6)
            kv = _rb(kv_acc[...])
            z = _rb(jnp.sum(z_acc[...], axis=1, keepdims=True))
            num = _rb(jnp.sum(phq * kv, axis=0, keepdims=True))
            den = _rb(_rb(jnp.sum(phq * z, axis=0, keepdims=True)) + 1e-6)
            o_ref[...] = (num / den).astype(o_ref.dtype)

    BH = B * H
    out = pl.pallas_call(
        kernel,
        grid=(BH, S // TS),
        in_specs=[
            pl.BlockSpec((None, 1, D), lambda i, j: (i, 0, 0)),
            pl.BlockSpec((None, TS, D), lambda i, j: (i, j, 0)),
            pl.BlockSpec((None, TS, D), lambda i, j: (i, j, 0)),
            pl.BlockSpec((M, D), lambda i, j: (0, 0)),
        ],
        out_specs=pl.BlockSpec((None, 1, D), lambda i, j: (i, 0, 0)),
        out_shape=jax.ShapeDtypeStruct((BH, 1, D), q.dtype),
        scratch_shapes=[pltpu.VMEM((M, D), _F32), pltpu.VMEM((M, 128), _F32)],
        compiler_params=pltpu.CompilerParams(
            dimension_semantics=("parallel", "arbitrary"),
            vmem_limit_bytes=64 * 1024 * 1024,
        ),
    )(q.reshape(BH, 1, D), k.reshape(BH, S, D), v.reshape(BH, S, D), omega)
    return out.reshape(B, H, 1, D)
```

```python
import jax
import jax.numpy as jnp
from jax import lax
import jax.experimental.pallas as pl
import jax.experimental.pallas.tpu as pltpu

_F32 = jnp.float32
_BF16 = jnp.bfloat16
_NT = (((1,), (1,)), ((), ()))

_C = 512
_SEG = _C // 2
_NB = 5

_HIGH = (
    (0, 0, 104, "B1m"),
    (0, 0, 104, "B4s"),
    (0, 1, 96, "B2m"),
    (1, 0, 88, "B4m"),
    (1, 0, 88, "B1s"),
    (1, 1, 88, "B2s"),
    (1, 1, 88, "B3s"),
)


def _piece_tables():
    low, high = {}, []
    for a in range(2):
        for sg in range(2):
            mine = [e for e in _HIGH if e[0] == a and e[1] == sg]
            n_low = _SEG - sum(e[2] for e in mine)
            assert n_low > 0 and n_low % 8 == 0
            low[(a, sg)] = (sg * _SEG, n_low)
            start = sg * _SEG + n_low
            for e in mine:
                high.append((a, sg, len(high), start, e[2], e[3]))
                start += e[2]
    return low, tuple(high)


_LOW_TAB, _HIGH_TAB = _piece_tables()


def _rb(x):
    return x.astype(_BF16).astype(_F32)


def _is_prev(e):
    return e[0] == 1 and e[5] != "B4m"


@jax.jit
def pallas_standalone__linear_kernel_rfa__decode_kernel(
    q: jax.Array,
    k: jax.Array,
    v: jax.Array,
    omega: jax.Array,
):
    B, H, Sq, D = q.shape
    S = k.shape[2]
    M = omega.shape[0]
    BH = B * H
    assert Sq == 1 and D == 256 and S % _C == 0
    NJ = S // _C
    NCH = BH * NJ
    assert NCH >= _NB
    scale = float(D) ** -0.25
    inv_sqrt_m = float(M) ** -0.5

    def kernel(q_hbm, k_hbm, v_hbm, om_hbm, o_ref,
               kbuf, vbuf, q_v, om_v, kv_acc, z_acc, o_acc, lsem, hsem, ssem):
        hbm = (k_hbm, v_hbm)
        buf = (kbuf, vbuf)

        def lo(a, sg, c, slot):
            st, n = _LOW_TAB[(a, sg)]
            return pltpu.make_async_copy(
                hbm[a].at[pl.ds(c * _C + st, n), :],
                buf[a].at[slot, pl.ds(st, n), :],
                lsem.at[a, slot, sg])

        def hi(e, c, slot):
            a, _, idx, st, n, _ = e
            return pltpu.make_async_copy(
                hbm[a].at[pl.ds(c * _C + st, n), :],
                buf[a].at[slot, pl.ds(st, n), :],
                hsem.at[slot, idx])

        omc = pltpu.make_async_copy(om_hbm, om_v, ssem.at[0])
        qc = pltpu.make_async_copy(q_hbm, q_v, ssem.at[1])
        omc.start()
        qc.start()
        for s in range(_NB):
            for a in range(2):
                for sg in range(2):
                    lo(a, sg, s, s).start(priority=1)
                    for e in _HIGH_TAB:
                        if e[0] == a and e[1] == sg and not (_is_prev(e) and s == _NB - 1):
                            hi(e, s, s).start(priority=1)
        omc.wait()
        qc.wait()

        def proj(kk):
            kp = lax.dot_general(om_v[...], kk, _NT, preferred_element_type=_F32)
            kf = kk.astype(_F32)
            sq = kf * kf
            sh = sq[:, :128] + sq[:, 128:]
            shi = sh.astype(_BF16)
            slo = (sh - shi.astype(_F32)).astype(_BF16)
            hl = jnp.concatenate([shi, slo], axis=1)
            ksq = lax.dot_general(jnp.ones((M, 256), _BF16), hl, _NT,
                                  preferred_element_type=_F32)
            return kp, ksq

        def feat(kp, ksq):
            kp = _rb(kp * scale)
            ksq = _rb(_rb(ksq * (scale * scale)) * 0.5)
            e = _rb(jnp.exp(_rb(kp - ksq)))
            phi = (_rb(e * inv_sqrt_m) + 1e-6).astype(_BF16)
            pf = phi.astype(_F32)
            zp = pf[:, 0:128]
            for t in range(1, kp.shape[1] // 128):
                zp = zp + pf[:, t * 128:(t + 1) * 128]
            return phi, zp

        def finish(i):
            rows = lax.broadcasted_iota(jnp.int32, (BH, D), 0)
            qf = jnp.sum(jnp.where(rows == i, q_v[...].astype(_F32), 0.0),
                         axis=0, keepdims=True)
            qs = qf * scale
            omf = om_v[...].astype(_F32)
            qp = _rb(jnp.sum(omf * qs, axis=1, keepdims=True))
            qsq = _rb(_rb(jnp.sum(qs * qs, axis=1, keepdims=True)) * 0.5)
            eq = _rb(jnp.exp(_rb(qp - qsq)))
            phq = _rb(_rb(eq * inv_sqrt_m) + 1e-6)
            z = _rb(jnp.sum(z_acc[...], axis=1, keepdims=True))
            den = _rb(_rb(jnp.sum(phq * z, axis=0, keepdims=True)) + 1e-6)
            num = _rb(jnp.sum(phq * _rb(kv_acc[...]), axis=0, keepdims=True))
            o_acc[pl.ds(i, 1), :] = num / den

        def body(c, carry):
            slot, i, j = carry
            pslot = jnp.where(slot == 0, _NB - 1, slot - 1)
            nxt = c + _NB

            @pl.when(j == 0)
            def _():
                kv_acc[...] = jnp.zeros_like(kv_acc)
                z_acc[...] = jnp.zeros_like(z_acc)

            def inject(label):
                for e in _HIGH_TAB:
                    if e[5] != label:
                        continue
                    if _is_prev(e):
                        @pl.when(nxt - 1 < NCH)
                        def _():
                            hi(e, nxt - 1, pslot).start(priority=0)
                    else:
                        @pl.when(nxt < NCH)
                        def _():
                            hi(e, nxt, slot).start(priority=0)

            def restart(a, sg):
                @pl.when(nxt < NCH)
                def _():
                    lo(a, sg, nxt, slot).start(priority=1)

            def wait_hi(a, sg):
                for e in _HIGH_TAB:
                    if e[0] == a and e[1] == sg:
                        hi(e, c, slot).wait()

            lo(0, 0, c, slot).wait()
            inject("B1s")
            wait_hi(0, 0)
            pa = proj(kbuf[slot, 0:_SEG, :])
            inject("B1m")
            restart(0, 0)

            lo(0, 1, c, slot).wait()
            inject("B2s")
            wait_hi(0, 1)
            pb = proj(kbuf[slot, _SEG:_C, :])
            phia, za = feat(*pa)
            inject("B2m")
            restart(0, 1)

            lo(1, 0, c, slot).wait()
            inject("B3s")
            wait_hi(1, 0)
            phib, zb = feat(*pb)
            z_acc[...] += za + zb

            lo(1, 1, c, slot).wait()
            inject("B4s")
            wait_hi(1, 1)
            phi = jnp.concatenate([phia, phib], axis=1)
            kv_acc[...] += jnp.dot(phi, vbuf[slot], preferred_element_type=_F32)
            inject("B4m")
            restart(1, 0)
            restart(1, 1)

            last = j == NJ - 1

            @pl.when(last)
            def _():
                finish(i)

            return (jnp.where(slot == _NB - 1, 0, slot + 1),
                    jnp.where(last, i + 1, i),
                    jnp.where(last, 0, j + 1))

        lax.fori_loop(0, NCH, body, (jnp.int32(0), jnp.int32(0), jnp.int32(0)))
        o_ref[...] = o_acc[...].astype(o_ref.dtype)

    out = pl.pallas_call(
        kernel,
        in_specs=[pl.BlockSpec(memory_space=pl.ANY)] * 4,
        out_specs=pl.BlockSpec(memory_space=pltpu.VMEM),
        out_shape=jax.ShapeDtypeStruct((BH, D), q.dtype),
        scratch_shapes=[
            pltpu.VMEM((_NB, _C, D), _BF16),
            pltpu.VMEM((_NB, _C, D), _BF16),
            pltpu.VMEM((BH, D), _BF16),
            pltpu.VMEM((M, D), _BF16),
            pltpu.VMEM((M, D), _F32),
            pltpu.VMEM((M, 128), _F32),
            pltpu.VMEM((BH, D), _F32),
            pltpu.SemaphoreType.DMA((2, _NB, 2)),
            pltpu.SemaphoreType.DMA((_NB, len(_HIGH_TAB))),
            pltpu.SemaphoreType.DMA((2,)),
        ],
        compiler_params=pltpu.CompilerParams(vmem_limit_bytes=32 * 1024 * 1024),
    )(q.reshape(BH, D), k.reshape(BH * S, D), v.reshape(BH * S, D), omega)
    return out.reshape(B, H, 1, D)
```

```python
import jax
import jax.numpy as jnp
from jax import lax
import jax.experimental.pallas as pl
import jax.experimental.pallas.tpu as pltpu

_F32 = jnp.float32
_BF16 = jnp.bfloat16
_NT = (((1,), (1,)), ((), ()))

_U = 512
_NB = 6
_TAIL_UNITS = 4
_SHIFT = (48, 48)

_PIECES = (
    (40, 120, 48, 48, 40, 32, 24, 56, 16, 88),
    (24, 16, 32, 24, 72, 56, 64, 40, 88, 96),
)
_ORDER = (
    (0, 0, 1, 0), (0, 1, 0, 0), (1, 8, 0, 0), (0, 4, 1, 1), (0, 6, 1, 0),
    (0, 5, 1, 0), (0, 9, 0, 1), (0, 7, 1, 0), (0, 8, 1, 0), (1, 9, 0, 2),
    (1, 2, 0, 0), (1, 3, 0, 0), (1, 4, 0, 0), (0, 2, 0, 0), (0, 3, 0, 0),
    (1, 0, 1, 0), (1, 1, 1, 0), (1, 7, 1, 0), (1, 5, 0, 1), (1, 6, 0, 1),
)
_STARTS = tuple(tuple(sum(p[:i]) for i in range(len(p))) for p in _PIECES)

assert all(sum(p) == _U for p in _PIECES)
assert sorted(o[:2] for o in _ORDER) == [
    (a, p) for a in range(2) for p in range(len(_PIECES[a]))]
assert all(_PIECES[a][-1] > _SHIFT[a] for a in range(2))
assert all(d >= 1 for a, p, _, d in _ORDER if p == len(_PIECES[a]) - 1)
assert all(d <= _NB - 3 for _, _, _, d in _ORDER)


def _rb(x):
    return x.astype(_BF16).astype(_F32)


def _compiler_params():
    kwargs = dict(vmem_limit_bytes=64 * 1024 * 1024)
    for name in ("disable_bounds_checks", "disable_semaphore_checks"):
        if hasattr(pltpu.CompilerParams, name):
            kwargs[name] = True
    return pltpu.CompilerParams(**kwargs)


@jax.jit
def pallas_standalone__linear_kernel_rfa__decode_kernel(
    q: jax.Array,
    k: jax.Array,
    v: jax.Array,
    omega: jax.Array,
):
    B, H, Sq, D = q.shape
    S = k.shape[2]
    M = omega.shape[0]
    BH = B * H
    assert Sq == 1 and D == 256 and S % _U == 0
    NJ = S // _U
    NU = BH * NJ
    assert NU >= _NB + _TAIL_UNITS
    scale = float(D) ** -0.25
    inv_sqrt_m = float(M) ** -0.5

    def kernel(q_hbm, k_hbm, v_hbm, om_hbm, o_ref,
               kbuf, vbuf, q_v, om_v, kv_acc, z_acc, o_acc, pq_s, sem, ssem):
        hbm = (k_hbm, v_hbm)
        buf = (kbuf, vbuf)

        def cp(a, u, slot, st, n):
            return pltpu.make_async_copy(
                hbm[a].at[pl.ds(u * _U + _SHIFT[a] + st, n), :],
                buf[a].at[slot, pl.ds(st, n), :],
                sem.at[a, slot])

        omc = pltpu.make_async_copy(om_hbm, om_v, ssem.at[0])
        qc = pltpu.make_async_copy(q_hbm, q_v, ssem.at[1])
        heads = [
            pltpu.make_async_copy(
                hbm[a].at[pl.ds(0, _SHIFT[a]), :],
                buf[a].at[_NB - 1, pl.ds(_U - _SHIFT[a], _SHIFT[a]), :],
                ssem.at[2 + a])
            for a in range(2)
        ]
        omc.start()
        qc.start()
        for hc in heads:
            hc.start()
        delay = {(a, p): d for a, p, _, d in _ORDER}
        for s in range(_NB):
            for a in range(2):
                for p, n in enumerate(_PIECES[a]):
                    if s < _NB - delay[(a, p)]:
                        cp(a, s, s, _STARTS[a][p], n).start(priority=1)
        omc.wait()
        qc.wait()
        for hc in heads:
            hc.wait()

        def phi_of(kk):
            kp = lax.dot_general(om_v[...], kk, _NT, preferred_element_type=_F32)
            kf = kk.astype(_F32)
            sq = kf * kf
            sh = sq[:, :128] + sq[:, 128:]
            shi = sh.astype(_BF16)
            slo = (sh - shi.astype(_F32)).astype(_BF16)
            hl = jnp.concatenate([shi, slo], axis=1)
            ksq = lax.dot_general(jnp.ones((M, 256), _BF16), hl, _NT,
                                  preferred_element_type=_F32)
            kp = _rb(kp * scale)
            ksq = _rb(_rb(ksq * (scale * scale)) * 0.5)
            e = _rb(jnp.exp(_rb(kp - ksq)))
            phi = (_rb(e * inv_sqrt_m) + 1e-6).astype(_BF16)
            pf = phi.astype(_F32)
            zp = pf[:, 0:128]
            for t in range(1, _U // 128):
                zp = zp + pf[:, t * 128:(t + 1) * 128]
            return phi, zp

        def q_side(i):
            rows = lax.broadcasted_iota(jnp.int32, (BH, D), 0)
            qf = jnp.sum(jnp.where(rows == i, q_v[...].astype(_F32), 0.0),
                         axis=0, keepdims=True)
            qs = qf * scale
            omf = om_v[...].astype(_F32)
            qp = _rb(jnp.sum(omf * qs, axis=1, keepdims=True))
            qsq = _rb(_rb(jnp.sum(qs * qs, axis=1, keepdims=True)) * 0.5)
            eq = _rb(jnp.exp(_rb(qp - qsq)))
            phq = _rb(_rb(eq * inv_sqrt_m) + 1e-6)
            z = _rb(jnp.sum(z_acc[...], axis=1, keepdims=True))
            den = _rb(_rb(jnp.sum(phq * z, axis=0, keepdims=True)) + 1e-6)
            pq_s[0:M, :] = jnp.broadcast_to(phq, (M, D))
            pq_s[M:M + 8, :] = jnp.broadcast_to(den, (8, D))

        def finish(i):
            num = _rb(jnp.sum(pq_s[0:M, :] * _rb(kv_acc[...]), axis=0, keepdims=True))
            o_acc[pl.ds(i, 1), :] = num / pq_s[M:M + 1, :]

        def unit_rows(a, slot):
            s = _SHIFT[a]
            prev = jnp.where(slot == 0, _NB - 1, slot - 1)
            return jnp.concatenate(
                [buf[a][prev, _U - s:_U, :], buf[a][slot, 0:_U - s, :]], axis=0)

        def wait_unit(a, c, slot):
            @pl.when(c < NU - 1)
            def _():
                cp(a, c, slot, 0, _U).wait()

            @pl.when(c == NU - 1)
            def _():
                cp(a, c, slot, 0, _U - _SHIFT[a]).wait()

        def body(c, carry):
            slot, i, j = carry
            last = j == NJ - 1

            @pl.when(j == 0)
            def _():
                kv_acc[...] = jnp.zeros_like(kv_acc)
                z_acc[...] = jnp.zeros_like(z_acc)

            wait_unit(0, c, slot)
            phi, zp = phi_of(unit_rows(0, slot))
            z_acc[...] += zp

            @pl.when(last)
            def _():
                q_side(i)

            wait_unit(1, c, slot)
            kv_acc[...] += jnp.dot(phi, unit_rows(1, slot),
                                   preferred_element_type=_F32)

            for a, p, prio, d in _ORDER:
                tgt = c - d + _NB
                ts = slot - d
                ts = jnp.where(ts < 0, ts + _NB, ts)

                @pl.when(tgt < NU - _TAIL_UNITS)
                def _():
                    cp(a, tgt, ts, _STARTS[a][p], _PIECES[a][p]).start(priority=prio)

            tgt = c - 1 + _NB
            ts = slot - 1
            ts = jnp.where(ts < 0, ts + _NB, ts)

            @pl.when((tgt >= NU - _TAIL_UNITS) & (tgt < NU - 1))
            def _():
                for a in range(2):
                    cp(a, tgt, ts, 0, _U).start(priority=1)

            @pl.when(tgt == NU - 1)
            def _():
                for a in range(2):
                    cp(a, tgt, ts, 0, _U - _SHIFT[a]).start(priority=1)

            @pl.when(last)
            def _():
                finish(i)

            return (jnp.where(slot + 1 == _NB, 0, slot + 1),
                    jnp.where(last, i + 1, i),
                    jnp.where(last, 0, j + 1))

        lax.fori_loop(0, NU, body, (jnp.int32(0), jnp.int32(0), jnp.int32(0)))
        o_ref[...] = o_acc[...].astype(o_ref.dtype)

    out = pl.pallas_call(
        kernel,
        in_specs=[pl.BlockSpec(memory_space=pl.ANY)] * 4,
        out_specs=pl.BlockSpec(memory_space=pltpu.VMEM),
        out_shape=jax.ShapeDtypeStruct((BH, D), q.dtype),
        scratch_shapes=[
            pltpu.VMEM((_NB, _U, D), _BF16),
            pltpu.VMEM((_NB, _U, D), _BF16),
            pltpu.VMEM((BH, D), _BF16),
            pltpu.VMEM((M, D), _BF16),
            pltpu.VMEM((M, D), _F32),
            pltpu.VMEM((M, 128), _F32),
            pltpu.VMEM((BH, D), _F32),
            pltpu.VMEM((M + 8, D), _F32),
            pltpu.SemaphoreType.DMA((2, _NB)),
            pltpu.SemaphoreType.DMA((4,)),
        ],
        compiler_params=_compiler_params(),
    )(q.reshape(BH, D), k.reshape(BH * S, D), v.reshape(BH * S, D), omega)
    return out.reshape(B, H, 1, D)
```
